```python
import os as _os
_os.environ.setdefault('JAX_PLATFORMS', 'cpu')
import jax
import jax.numpy as jnp

def _softmax(x, axis=-1):
    return jax.nn.softmax(x, axis=axis)

def _gelu(x):
    return jax.nn.gelu(x, approximate=True)

def _silu(x):
    return jax.nn.silu(x)

def _sigmoid(x):
    return jax.nn.sigmoid(x)

def _layernorm(x, axis=-1, eps=1e-05):
    m = jnp.mean(x, axis=axis, keepdims=True)
    v = jnp.var(x, axis=axis, keepdims=True)
    return (x - m) / jnp.sqrt(v + eps)

def _scatter_add(tgt, idx, src, axis=0):
    return tgt.at[idx].add(src)

def _segment_sum(src, seg, n):
    return jax.ops.segment_sum(src, seg, n)

class _Rng:

    def __init__(self, key):
        self._k = key

    def _next(self):
        self._k, sub = jax.random.split(self._k)
        return sub

    def normal(self, shape):
        return jax.random.normal(self._next(), shape, dtype=jnp.bfloat16)

    def randint(self, lo, hi, shape):
        return jax.random.randint(self._next(), shape, lo, hi, dtype=jnp.int32)

    def uniform(self, shape, lo=0.0, hi=1.0):
        return jax.random.uniform(self._next(), shape, jnp.bfloat16, lo, hi)

    def permutation(self, n):
        return jax.random.permutation(self._next(), n)
kernel_name = 'sequential_preLN__memory_aug_recurrent_mem_tr__mixer_token_mlp__prompt'

def setup_inputs():
    _rng = _Rng(jax.random.key(int.from_bytes(__import__("os").urandom(4), "little")))
    _w = lambda a: (lambda t: t.astype(jnp.bfloat16) if jnp.issubdtype(t.dtype, jnp.floating) else t)(jnp.asarray(a))

    def _A_setup():
        B, S, Dm = (1, 2048, 448)
        H, Dh = (16, 256)
        M, seg = (8, 32)
        seg = min(seg, S)
        S = S // seg * seg
        return {'x': _w((lambda *s: _rng.normal(s) * 0.05)(B, S, Dm)), 'mem0': _w((lambda *s: _rng.normal(s) * 0.2)(B, M, Dm)), 'Wq': _w((lambda *s: _rng.normal(s) * 1.6)(Dm, H, Dh) * Dm ** (-0.5)), 'Wk': _w((lambda *s: _rng.normal(s) * 1.6)(Dm, H, Dh) * Dm ** (-0.5)), 'Wv': _w((lambda *s: _rng.normal(s) * 0.2)(Dm, H, Dh) * Dm ** (-0.5)), 'Wo': _w((lambda *s: _rng.normal(s) * 0.2)(H, Dh, Dm) * (H * Dh) ** (-0.5)), 'seg_len': seg}
    _A_in = _A_setup()

    def _B_setup():
        B, S, D, F = (1, 2048, 448, 1792)
        return {'x': _w((lambda *s: _rng.normal(s) * 0.05)(B, S, D)), 'w1': _w((lambda *s: _rng.normal(s) * 0.2)(S, F) * S ** (-0.5)), 'b1': _w((lambda *s: _rng.normal(s) * 0.2)(F) * 0.02), 'w2': _w((lambda *s: _rng.normal(s) * 0.2)(F, S) * F ** (-0.5)), 'b2': _w((lambda *s: _rng.normal(s) * 0.05)(S) * 0.02)}
    _B_in = _B_setup()
    return {'A_x': _A_in['x'], 'A_mem0': _A_in['mem0'], 'A_Wq': _A_in['Wq'], 'A_Wk': _A_in['Wk'], 'A_Wv': _A_in['Wv'], 'A_Wo': _A_in['Wo'], 'A_seg_len': _A_in['seg_len'], 'B_x': _B_in['x'], 'B_w1': _B_in['w1'], 'B_b1': _B_in['b1'], 'B_w2': _B_in['w2'], 'B_b2': _B_in['b2']}

def reference(A_x, A_mem0, A_Wq, A_Wk, A_Wv, A_Wo, A_seg_len, B_x, B_w1, B_b1, B_w2, B_b2):

    def _A_ref(x, mem0, Wq, Wk, Wv, Wo, seg_len):
        B, S, Dm = x.shape
        H, Dh = (Wq.shape[1], Wq.shape[2])
        M = mem0.shape[1]
        scale = Dh ** (-0.5)
        n_seg = S // seg_len
        L = M + seg_len
        idx = jnp.arange(L)
        mask = (idx[:, None] < M) | (idx[:, None] >= idx[None, :])
        mem = mem0
        outs = []
        for s in range(n_seg):
            xs = x[:, s * seg_len:(s + 1) * seg_len, :].copy()
            h = jnp.concatenate([mem, xs], axis=1)
            q = jnp.einsum('btd,dhe->bhte', h, Wq)
            k = jnp.einsum('btd,dhe->bhte', h, Wk)
            v = jnp.einsum('btd,dhe->bhte', h, Wv)
            scores = jnp.einsum('bhqe,bhke->bhqk', q, k) * scale
            scores = jnp.where(mask[None, None], scores, -1000000000.0)
            p = _softmax(scores, axis=-1)
            o = jnp.einsum('bhqk,bhke->bhqe', p, v)
            o = jnp.einsum('bhte,hed->btd', o, Wo)
            mem = o[:, :M, :].copy()
            outs.append(o[:, M:, :])
        return jnp.concatenate(outs, axis=1)

    def _B_ref(x, w1, b1, w2, b2):
        B, S, D = x.shape
        h = _layernorm(x, axis=-1)
        u = jnp.einsum('bsd,sf->bdf', h, w1) + b1
        u = _gelu(u)
        y = jnp.einsum('bdf,fs->bds', u, w2) + b2
        return (lambda x, *d: x.transpose(*d))(y, 0, 2, 1)
    x = A_x
    h = x + _A_ref(_layernorm(x, axis=-1), A_mem0, A_Wq, A_Wk, A_Wv, A_Wo, A_seg_len)
    h2 = h + _B_ref(_layernorm(h, axis=-1), B_w1, B_b1, B_w2, B_b2)
    return h2
```

```python
import functools
import itertools
from typing import NamedTuple

import jax
import jax.numpy as jnp
from jax import lax
import jax.experimental.pallas as pl
import jax.experimental.pallas.tpu as pltpu

F32 = jnp.float32
BF16 = jnp.bfloat16
U32 = jnp.uint32
LANE = 128
HALF = 64
EPS = 1e-5
NEG = -1000000000.0
LOG2E = 1.4426950408889634
GELU_A = 0.7978845608028654
GELU_B = GELU_A * 0.044715

_PASSES = (
    ".+...... ++...... ....+...+--... +-..-+........",
    "+-...... +....... -.+.....+..-.. +.-+....-.....",
    "...+.... ...+.... -++-.......... ...+....-+..-.",
    "..+..... ..+..... .+..+-....-... .-...+...+-...",
    "....-+.. .....+.. ....+....-..+- ....-++-......",
    "....+... ....++.. ..+...-....-+. ..-+..+....-..",
    ".......+ ......++ ....+-.+.....- .....+.-..-..+",
    "......+- ......+. ..+-..-+...... ...+.......--+",
    "-+-+.... .+.+.... +...-......... .....-..+.....",
    "+.+..... ++++.... ..-.......+... .+.-..........",
    "+-+..... ++.+.... +.........-... .-......+.....",
    ".+...+.. .+...+.. ....-....+.... ....+-........",
    "+...+... +...+... ..-........+.. ..+-..........",
    ".+..+... +....-.. ..+.-....+.-.. ..-++-........",
    "..-+..-+ ...+...+ ..-+.......... ...-........+.",
    "..+...+. ..++..++ ....-+........ .....-....+...",
    "..+...+- ...+..++ ..-++-........ ...-.+....-.+.",
    ".....+.+ .....+.+ ..-..........+ ...-...+......",
    "....+.+. ....+.+. ....-.+....... .....-.....+..",
    "....+..+ .....+-. ......+......- .......-...+..",
    ".+.+.+.+ ++++++++ ..+........... ...+..........",
    "+-+-+-+- +.+.+.+. ....+......... .....+........",
    "+-+-.-.- +++++.+. ..+.-......... ...+.-........",
)
_MIXED = (
    (".............+..+...+.......", ".............+......+...-...", "........+........+.......+..",
     ".......+..............+...+.", ".......+..........-...+.....", "..+................-.......-"),
    (".............+..+.......-...", "........+........+...-......", "........+............-...+..",
     ".......+..........-.......+.", "..+....................-...-", "..+................-...-...."),
)
_SIGN = {"+": 1, "-": -1, ".": 0}


def _shared_sums(matrix):
    rows = [{i: v for i, v in enumerate(r) if v} for r in matrix]
    n, steps = len(matrix[0]), []
    while True:
        count = {}
        for r in rows:
            for a, b in itertools.combinations(sorted(r), 2):
                count[a, b, r[a] * r[b]] = count.get((a, b, r[a] * r[b]), 0) + 1
        key, c = max(sorted(count.items()), key=lambda kv: kv[1], default=(None, 0))
        if c < 2:
            return steps, rows
        a, b, s = key
        steps.append((n, a, b, s))
        for r in rows:
            if a in r and b in r and r[a] * r[b] == s:
                r[n] = r.pop(a)
                del r[b]
        n += 1


class _SignedSums:
    def __init__(self, matrix):
        self.steps, self.rows = _shared_sums(matrix)
        self.known = {}
        self.acc = [None] * len(self.rows)
        self.taken = []

    def feed(self, i, value):
        self.known[i] = value
        for n, a, b, s in self.steps:
            if n not in self.known and a in self.known and b in self.known:
                self.known[n] = self.known[a] + self.known[b] if s > 0 else self.known[a] - self.known[b]
        for k, r in enumerate(self.rows):
            for v in sorted((v for v in r if v in self.known), key=lambda v: -r[v]):
                s = r.pop(v)
                if self.acc[k] is None:
                    self.acc[k] = (s, self.known[v])
                elif self.acc[k][0] > 0:
                    self.acc[k] = (1, self.acc[k][1] + self.known[v] if s > 0 else self.acc[k][1] - self.known[v])
                else:
                    self.acc[k] = (1, self.known[v] - self.acc[k][1]) if s > 0 else (-1, self.acc[k][1] + self.known[v])

    def finished(self):
        new = [k for k, r in enumerate(self.rows) if not r and k not in self.taken]
        self.taken += new
        return [(k, self.acc[k][1] if self.acc[k][0] > 0 else -self.acc[k][1]) for k in new]

    def result(self):
        return [v if s > 0 else -v for s, v in self.acc]


def _signed_sums(matrix, values):
    sums = _SignedSums(matrix)
    for i, v in enumerate(values):
        sums.feed(i, v)
    return sums.result()


_LHS = [[_SIGN[c] for c in p.split()[0]] for p in _PASSES]
_OUT = [[_SIGN[p.split()[1][o]] for p in _PASSES] for o in range(8)]
_AHEAD = (0, 2, 6, 11, 17)
assert not any(v for t in _AHEAD for v in _LHS[t][0::2])
_RHS = [[[_SIGN[c] for c in p.split()[2 + half]] for p in _PASSES] for half in range(2)]


class _Plan(NamedTuple):
    key_tiles: tuple
    value_tiles: tuple
    score_tiles: tuple
    pair_passes: tuple
    values_before_scores: tuple


_FIRST = _Plan((0, 3, 2, 1), (3, 2, 0, 1), (4, 3, 1, 2, 0), (0, 1, 2, 3, 4, 5, 6), (6, 4, 4, 4))
_LATER = _Plan((2, 0, 3, 1), (1, 0, 2, 3), (3, 1, 2, 4, 0), (6, 2, 0, 1, 4, 5, 3), (4, 4, 4, 4))

_NN = (((1,), (0,)), ((), ()))
_NT = (((1,), (1,)), ((), ()))


def _dot(a, b, dims=_NN):
    return lax.dot_general(a, b, dims, preferred_element_type=F32)


def _pack(v):
    return pltpu.bitcast(v.astype(BF16), U32)


def _unpack(w):
    return pltpu.bitcast(w, BF16)


def _low_half(rows):
    return lax.broadcasted_iota(jnp.int32, (rows, LANE), 1) < HALF


def _drain(work):
    for _ in work:
        pass


def _gelu(x, factor):
    half = x * (0.5 * factor)
    return half + half * jnp.tanh(x * (GELU_A + GELU_B * (x * x)))


def _tree_sum(values):
    while len(values) > 1:
        values = [values[i] + values[i + 1] if i + 1 < len(values) else values[i] for i in range(0, len(values), 2)]
    return values[0]


def _column_mean(blocks):
    total, n = None, 0
    for get in blocks:
        t = get()
        part = _tree_sum([t[r:r + 8] for r in range(0, t.shape[0], 8)])
        total, n = part if total is None else total + part, n + t.shape[0]
        yield total
    return jnp.sum(total, axis=0, keepdims=True) * (1.0 / n)


def _kernel(xt_hbm, mem_ref, wq_hbm, wk_hbm, wv_hbm, wot_hbm, w1_hbm, b1_ref, w2_hbm, b2_ref,
            out_hbm,
            xt_v, wq_v, wk_v, wv_v, wot_v, w1_v, w2_v, wp_s, wh_s, wa_s, wc_s,
            xn_s, ht_s, hl_s, a_s, pre_s, tl_s, k_s, v_s, lq_s, g_s, out_v, sems,
            *, S, D, H, E, M, SEG, F):
    assert (D, E, M, SEG, H) == (7 * HALF, 2 * LANE, 8, 32, 16) and S == 16 * LANE and F == 14 * LANE
    DF = (D // LANE) * LANE
    NF = DF // LANE
    NC = NF + 1
    NB = D // HALF
    NP = H // 2
    NTILE = NF * H + NP
    G = LANE // SEG
    NG = S // LANE
    TPS = SEG // 8
    scale = float(E) ** -0.5
    FB = F // NB

    def rows_of(start, n):
        return pl.ds(start if isinstance(start, int) else pl.multiple_of(start, 8), n)

    def lanes_of(t):
        return slice(t * LANE, (t + 1) * LANE)

    def cp_heads(src, dst, j, sem):
        return pltpu.make_async_copy(src.bitcast(U32).at[:, j, :], dst.at[j], sems.at[sem])

    def cp_keys(j):
        return [cp_heads(wq_hbm, wq_v, j, j), cp_heads(wk_hbm, wk_v, j, j)]

    def cp_values(j):
        return [cp_heads(wv_hbm, wv_v, j, NP + j),
                pltpu.make_async_copy(wot_hbm.at[pl.ds(2 * j, 2)], wot_v.at[pl.ds(2 * j, 2)], sems.at[NP + j])]

    def wait_all(copies):
        for cp in copies:
            cp.wait()

    def cp_block(src, dst, rows, cols, sem):
        block = (pl.ds(rows[0], rows[1] - rows[0]), pl.ds(cols[0], cols[1] - cols[0]))
        return pltpu.make_async_copy(src.at[block], dst.at[block], sems.at[2 * NP + sem])

    LATE = 4
    KB = S // 4
    cp_x0 = cp_block(xt_hbm, xt_v, (0, D), (0, 2 * LANE), 0)
    cp_early = [cp_block(xt_hbm, xt_v, (0, D), (2 * LANE, (LATE + 2) * LANE), 1), cp_block(w2_hbm, w2_v, (0, F), (0, KB), 1)]
    cp_early += [cp_block(w1_hbm, w1_v, (j * KB, j * KB + LATE * SEG), (0, F), 1) for j in range(4)]
    cp_late = [cp_block(xt_hbm, xt_v, (0, D), ((LATE + 2) * LANE, S), 2), cp_block(w2_hbm, w2_v, (0, F), (KB, S), 2)]
    cp_late += [cp_block(w1_hbm, w1_v, (j * KB + LATE * SEG, (j + 1) * KB), (0, F), 2) for j in range(4)]

    lane = lax.broadcasted_iota(jnp.int32, (8, LANE), 1)
    causal = (lane & 7) <= lax.broadcasted_iota(jnp.int32, (8, LANE), 0)

    def block(i):
        return slice(i * HALF, (i + 1) * HALF)

    def hold(ref, v):
        n = 8 * (4 // ref.dtype.itemsize)
        ref[ref.shape[0] - n:, 0:LANE] = jnp.broadcast_to(v, (n, LANE)).astype(ref.dtype)

    def chunk_of(ref, chunk):
        return ref.at[:, pl.ds(pl.multiple_of(chunk * LANE, LANE), LANE)]

    def prepare_tokens(chunk, slot):
        src = chunk_of(xt_v, chunk)
        x = lambda i: src[block(i), :].astype(F32)
        mean = yield from _column_mean(functools.partial(x, i) for i in range(NB))
        var = yield from _column_mean(functools.partial(lambda i: jnp.square(x(i) - mean), i) for i in range(NB))
        inv = lax.rsqrt(var + EPS)
        for c in range(NC):
            n = [(x(i) - mean) * inv for i in range(2 * c, min(2 * c + 2, NB))]
            t = jnp.concatenate([n[0], n[-1]], axis=0).T
            xn_s[rows_of(slot * LANE, LANE), lanes_of(c)] = t
            yield t[LANE - 8:]

    def head(w_v, h, c):
        u = w_v[h[0], :, lanes_of(c)]
        return pltpu.bitcast(u & jnp.uint32(0xFFFF0000) if h[1] else u << 16, F32)

    def put(pair, t, r, v):
        wp_s[rows_of(pair * HALF + r // 2, v.shape[0] // 2), lanes_of(t)] = _pack(v)

    def put_top(pair, e, v):
        put(pair, e, 0, v[:LANE])
        put(pair, 2 + e, 0, v[LANE:2 * LANE])

    def put_rest(pair, a, b):
        put(pair, 4, 0, jnp.concatenate([a[block(0)], a[block(2)] - b[block(2)]], axis=0))
        put(pair, 5, 0, jnp.concatenate([b[block(0)], b[block(1)] - a[block(1)]], axis=0))
        put(pair, 6, 0, jnp.concatenate([b[block(2)], a[block(1)]], axis=0))

    def fold(base, j, left, right):
        lo = _low_half(D)
        TOP = 2 * LANE
        both = lambda get, e, rows: jnp.concatenate([get((j, e), c)[rows] for c in range(2)], axis=1)
        third, last = [], []
        for e in range(2):
            r = [right((j, e), c) for c in range(2)]
            part = lambda i, c: r[c][block(i)]
            l0, l1 = left((j, e), 0), left((j, e), 1)
            pa = _dot(l0, jnp.concatenate([part(4, 0), part(6, 0) - part(6, 1)], axis=0), _NT)
            pb = _dot(l1, jnp.concatenate([part(4, 1), part(5, 1) - part(5, 0)], axis=0), _NT)
            pc = _dot(l0 + l1, jnp.concatenate([part(6, 1), part(5, 0)], axis=0), _NT)
            third.append(pb + jnp.where(lo, pa, pc))
            put_top(base + 2 * NP + j, e, third[e])
            last.append(jnp.where(lo, pc, pa))
        put_rest(base + 2 * NP + j, third[0][TOP:], third[1][TOP:])
        tile = jnp.where(lo, *last) + pltpu.roll(jnp.where(lo, last[1], last[0]), HALF, 1)
        put_top(base + NF * NP + j // 2, 0, tl_s[...])
        put_top(base + NF * NP + j // 2, 1, tile)
        put_rest(base + NF * NP + j // 2, tl_s[TOP:, :], tile[TOP:])
        tl_s[...] = tile
        rest = [_dot(both(left, e, slice(TOP, D)), both(right, e, slice(0, TOP)), _NT) for e in range(2)]
        for c in range(2):
            put_rest(base + c * NP + j, rest[0][:, lanes_of(c)], rest[1][:, lanes_of(c)])
        for e in range(2):
            top = _dot(both(left, e, slice(0, TOP)), both(right, e, slice(0, TOP)), _NT)
            for c in range(2):
                put_top(base + c * NP + j, e, top[:, lanes_of(c)])

    def prologue():
        folds = [cp for copies in (cp_keys, cp_values) for j in range(NP) for cp in copies(j)]
        for cp in [cp_x0] + folds + cp_early + cp_late:
            cp.start()
        cp_x0.wait()
        lax.fori_loop(0, 2, lambda c, _: _drain(prepare_tokens(c, c)), None)

        tl_s[...] = jnp.zeros(tl_s.shape, F32)

        def k_body(j, c):
            wait_all(cp_keys(j))
            fold(0, j, functools.partial(head, wk_v), functools.partial(head, wq_v))
            return c

        def v_body(j, left):
            wait_all(cp_values(j))
            fold(NTILE // 2, j, functools.partial(head, wv_v),
                 lambda h, c: wot_v[2 * h[0] + h[1], :, lanes_of(c)].astype(F32))
            return left - 1

        lax.fori_loop(0, NP, k_body, 0)
        return lax.fori_loop(0, NP, v_body, NP)

    def combine(entry, half, store):
        used = sorted({n for m in _MIXED[half] for n, c in enumerate(m) if c != "."})
        mixed = _SignedSums([[_SIGN[m[n]] for n in used] for m in _MIXED[half]])
        for k, n in enumerate(used):
            mixed.feed(k, entry(n // 4, n % 4))
            if k % 3 == 2:
                yield
        sums = _SignedSums(_RHS[half])
        for k, v in enumerate(mixed.result()):
            sums.feed(8 + k, v)
        for k in range(8):
            sums.feed(k, entry(half + 2 * (k // 4), k % 4))
            for t, v in sums.finished():
                store(t, _pack(v))
            yield

    def combine_folded(q, i, half):
        @functools.cache
        def part(p, t, h):
            return _unpack(wp_s[rows_of((2 * q + p) * HALF + h * HALF // 2 + 8 * i, 8), lanes_of(t)]).astype(F32)

        def entry(k, j):
            p, e = j // 2, j % 2
            if k < 5:
                return part(p, 2 * (k // 2) + e, k % 2)
            if k == 5:
                return part(p, 6, 1) if e == 0 else part(p, 5, 1) + part(p, 6, 1)
            return part(p, 4, 1) + part(p, 6, 0) if e == 0 else part(p, 6, 0)

        def store(t, w):
            wh_s[rows_of(q * HALF + half * HALF // 2 + 8 * i, 8), lanes_of(t)] = w
        return combine(entry, half, store)

    def combine_w2(n):
        q, r = n // 4, n % 4
        src = w2_v.at[pl.ds(pl.multiple_of(r * HALF, HALF), F - FB + HALF), pl.ds(pl.multiple_of(q * 4 * LANE, LANE), 4 * LANE)]
        dst = wc_s.at[rows_of(q * FB + r * HALF // 2, FB // 2 + HALF // 2), :]
        for i in range(HALF // 16):
            for half in range(2):
                @functools.cache
                def entry(k, j):
                    return src[k * FB + 16 * i:k * FB + 16 * i + 16, lanes_of(j)].astype(F32)

                def store(t, w):
                    dst[half * FB // 2 + 8 * i:half * FB // 2 + 8 * i + 8, lanes_of(t)] = w
                yield from combine(entry, half, store)

    def combine_w1(n):
        src = [w1_v.at[pl.ds(pl.multiple_of(j * KB + n * SEG, SEG), SEG), :] for j in range(4)]
        dst = wa_s.at[rows_of(n * SEG // 2, SEG // 2), :]
        for i in range(SEG // 16):
            for c in range(FB // LANE):
                for half in range(2):
                    @functools.cache
                    def entry(k, j):
                        return src[j][16 * i:16 * i + 16, lanes_of(k * FB // LANE + c)].astype(F32)

                    def store(t, w):
                        dst[8 * i:8 * i + 8, lanes_of(4 * t + 2 * half + c)] = w
                    yield from combine(entry, half, store)

    def group_allreduce(v, op):
        for d in (4, 2, 1):
            other = jnp.where((lane & d) != 0, pltpu.roll(v, d, 1), pltpu.roll(v, LANE - d, 1))
            v = op(v, other)
        return v

    def weight(ref, i, t, rows=HALF, paced=None):
        w = ref[rows_of(i * rows, rows), lanes_of(t)]
        return _unpack(w if paced is None else paced.tie(w))

    def pair_lhs(rows):
        lo = _low_half(rows.shape[0])
        t = [rows[:, c * LANE:(c + 1) * LANE] for c in range(NC)]
        out = [t[0], t[1], jnp.where(lo, t[2], t[3]), t[2], jnp.where(lo, t[3], t[2])]
        return [v.astype(BF16) for v in out] if rows.shape[0] % 16 == 0 else out

    def project_plain(lhs, q, between, plan):
        out = []
        for pair in (2 * q, 2 * q + 1):
            p = [None] * 7
            for t in plan.pair_passes:
                p[t] = between(_dot(lhs[(0, 0, 1, 1, 2, 3, 4)[t]], weight(wp_s, pair, t, paced=between)))
            out += [p[0] + p[2] + p[4] + p[6], p[1] + p[3] + p[5] + p[6]]
        return out

    def quad_nodes(rows):
        lo = _low_half(rows.shape[0])
        t = [rows[:, lanes_of(c)] for c in range(NC)]
        sw = pltpu.roll(t[2], HALF, 1)
        x4, x5, x6 = 0.5 * jnp.where(lo, t[2], sw), 0.5 * jnp.where(lo, sw, t[2]), 0.5 * t[3]
        return [jnp.where(lo, x4 + x5 + x6, t[0]), jnp.where(lo, t[0], x4 - x5 - x6),
                jnp.where(lo, x5 - x4 - x6, t[1]), jnp.where(lo, t[1], x6 - x4 - x5)]

    def project_quad(lhs, q, between):
        sums = _SignedSums(_OUT)
        for t in (0, 1, 2, 3, 8, 9, 10, 20, 21, 22, 17, 11, 18, 4, 12, 5, 13, 19, 6, 14, 7, 15, 16):
            if t in _AHEAD:
                sums.feed(t, pre_s[q * SEG:(q + 1) * SEG, lanes_of(_AHEAD.index(t))])
            else:
                sums.feed(t, between(_dot(lhs(t), weight(wh_s, q, t, paced=between))))
        out = sums.result()
        return [jnp.concatenate([out[2 * j], out[2 * j + 1]], axis=0) for j in range(4)]

    def stage(dst, tiles, q, slots):
        c = min(4 * q // H, NF)
        for r, slot in enumerate(slots):
            rows = []
            for tile in tiles:
                blk = tile[8 * r:8 * r + 8]
                rows += [blk] if c < NF else [jnp.where(lane < HALF, blk, 0.0), jnp.where(lane < HALF, 0.0, blk)]
            r0 = slot * HALF + (q - c * H // 4) * 4 * len(rows)
            dst[r0:r0 + 4 * len(rows), lanes_of(c)] = _pack(jnp.concatenate(rows, axis=0))

    def quad_order(order):
        return [q for c in order for q in range(c * H // 4, min((c + 1) * H, NTILE) // 4)]

    def live_rows(t):
        return [i for i in range(TPS + 1) if i == 0 or i >= t]

    def attend(i, mem, project, first, count, keys, plan):
        slots = [G * TPS + i] + list(range(first, first + count))
        seen = [G * TPS + i] + list(range(i * TPS, (i + 1) * TPS))
        for q in quad_order(plan.key_tiles):
            stage(k_s, project(q), q, slots)
        for t in slots:
            keys[t] = _unpack(pltpu.bitcast(_unpack(k_s[t * HALF:(t + 1) * HALF, :]).T, U32))
        early = plan.values_before_scores[i]
        for q in quad_order(plan.value_tiles)[:early]:
            stage(v_s, project(NTILE // 4 + q), q, slots)

        hs = jnp.concatenate([mem, xn_s[i * SEG:(i + 1) * SEG, :]], axis=0)
        sc = {}
        for t in plan.score_tiles:
            rows = live_rows(t)
            r = _dot(jnp.concatenate([hs[8 * b:8 * b + 8] for b in rows], axis=0), keys[seen[t]])
            for n, b in enumerate(rows):
                sc[b, t] = r[8 * n:8 * n + 8]
        prob = {}
        for b in range(TPS + 1):
            nvalid = TPS + 1 if b == 0 else b + 1
            tiles = [sc[b, t] for t in range(nvalid)]
            if b > 0:
                tiles[b] = jnp.where(causal, tiles[b], NEG / scale)
            mx = group_allreduce(functools.reduce(jnp.maximum, tiles), jnp.maximum)
            ex = [jnp.exp2((t - mx) * (scale * LOG2E)) for t in tiles]
            inv = 1.0 / group_allreduce(functools.reduce(jnp.add, ex), jnp.add)
            for t in range(nvalid):
                prob[b, t] = ex[t] * inv

        for q in quad_order(plan.value_tiles)[early:]:
            stage(v_s, project(NTILE // 4 + q), q, slots)
        cols = [None] * NC
        for c in plan.value_tiles:
            acc = {}
            for t in range(TPS + 1):
                rows = live_rows(t)
                r = _dot(jnp.concatenate([prob[b, t] for b in rows], axis=0), weight(v_s, seen[t], c))
                for n, b in enumerate(rows):
                    acc[b] = r[8 * n:8 * n + 8] if b not in acc else acc[b] + r[8 * n:8 * n + 8]
            cols[c] = jnp.concatenate([acc[b] for b in range(TPS + 1)], axis=0)
        cols[NF] = cols[NF] + pltpu.roll(cols[NF], HALF, 1)
        o = jnp.concatenate(cols, axis=1)
        a_s[i * SEG:(i + 1) * SEG, :] = o[M:]
        return o[:M]

    def normalise(chunk):
        x, res, dst = (chunk_of(ref, chunk) for ref in (xt_v, ht_s, hl_s))
        attn = [a_s[:, lanes_of(c)].T for c in range(NC)]
        yield

        def residual(i):
            h = x[block(i), :].astype(F32) + attn[i // 2][block(i % 2)]
            res[block(i), :] = h
            return h
        mean = yield from _column_mean(functools.partial(residual, i) for i in range(NB))
        var = yield from _column_mean(
            functools.partial(lambda i: jnp.square(res[block(i), :] - mean), i) for i in range(NB))
        r1 = lax.rsqrt(var + EPS)
        inv = r1 * lax.rsqrt(var * r1 * r1 + EPS)
        for i in range(NB):
            v = (res[block(i), :] - mean) * inv
            dst[block(i), :] = v
            yield v[HALF - 8:]

    def stage_quad_lhs(mem):
        n = SEG - M
        nodes = [quad_nodes(jnp.concatenate([mem, xn_s[LANE:LANE + n, :]], axis=0)),
                 quad_nodes(xn_s[LANE + n:LANE + n + SEG, :])]
        for t, v in enumerate(_signed_sums(_LHS, [nodes[l][i] for i in range(4) for l in range(2)])):
            if t not in _AHEAD:
                lq_s[:, lanes_of(t)] = _pack(v)

    def ahead_lhs():
        nodes = quad_nodes(xn_s[LANE + SEG - M:LANE + 2 * SEG - M, :])
        return [v.astype(BF16) for v in _signed_sums([_LHS[t][1::2] for t in _AHEAD], nodes)]

    def work_ahead(part, lhs):
        for r in range(NTILE // 2 // G):
            q = part * (NTILE // 2 // G) + r
            for n, t in enumerate(_AHEAD):
                pre_s[rows_of(q * SEG, SEG), lanes_of(n)] = _dot(lhs[n], weight(wh_s, q, t))

    def next_chunk():
        xn_s[0:LANE, :] = xn_s[LANE:2 * LANE, :]
        xn_s[LANE:2 * LANE, :] = xn_s[2 * LANE:, :]

    class Paced:
        def __init__(self, keep):
            self.work, self.keep, self.due = None, keep, None

        def tie(self, w):
            if self.due is None:
                return w
            v, self.due = pltpu.bitcast(self.due, U32), None
            return jnp.concatenate([w[:-8], jnp.where(self.keep, w[-8:], v)], axis=0)

        def start(self, work, every, *refs):
            self.work, self.every, self.refs, self.count = work, every, refs, 0

        def finish(self):
            _drain(self.work or ())
            self.work = None

        def __call__(self, result):
            if self.work is not None:
                self.count += 1
                if self.count % self.every == 0:
                    for ref in self.refs:
                        hold(ref, result[:8 * (4 // ref.dtype.itemsize)])
                    self.due = next(self.work, self)
                    if self.due is self:
                        self.work, self.due = None, None
            return result

    def first_group():
        m0 = mem_ref[0].astype(F32)
        mem = jnp.concatenate([m0[:, :DF], m0[:, DF:], m0[:, DF:]], axis=1)
        paced = Paced(None)
        for i in range(G):
            lhs = pair_lhs(jnp.concatenate([mem, xn_s[i * SEG:(i + 1) * SEG, :]], axis=0))
            work = itertools.chain.from_iterable(
                combine_folded(q, r, half) for q in range(i * NTILE // 2 // G, (i + 1) * NTILE // 2 // G)
                for r in range(HALF // 16) for half in range(2))
            paced.start((None for _ in zip(work, work)), 1)
            project = functools.partial(project_plain, lhs, between=paced, plan=_FIRST)
            mem = attend(i, mem, project, i * TPS, TPS, {}, _FIRST)
            paced.finish()
            _drain(work)
        stage_quad_lhs(mem)
        return mem

    def group(zero, g, mem):
        pl.when(g == LATE)(lambda: wait_all(cp_late))
        next_chunk()
        early = ahead_lhs()
        paced = Paced(lane >= zero)
        keys = {}
        done = 0
        late_norm = normalise(g - 1)
        next(late_norm)
        for i in range(G):
            n = SEG - M
            if i == 0:
                project = functools.partial(project_quad, lambda t: _unpack(lq_s[:, lanes_of(t)]), between=paced)
                n += SEG
            else:
                lhs = pair_lhs(jnp.concatenate([mem, xn_s[done:done + n, :]], axis=0))
                project = functools.partial(project_plain, lhs, between=paced, plan=_LATER)
            if i == 0:
                paced.start(combine_w1(g), 4, w1_v)
            elif i == 1:
                paced.start(combine_w2(g), 4, w2_v)
            elif i == 2:
                paced.start(prepare_tokens(jnp.minimum(g + 2, NG - 1), 2), 20)
            else:
                paced.start(late_norm, 10)
            mem = attend(i, mem, project, done // 8, n // 8, keys, _LATER)
            done += n
            paced.finish()
            work_ahead(i, early)
        stage_quad_lhs(mem)
        return mem

    def before_groups(zero):
        @pl.when(zero == 0)
        def _():
            wait_all(cp_early)
            _drain(prepare_tokens(2, 2))
            _drain(combine_w1(0))
            lhs = ahead_lhs()
            for part in range(G):
                work_ahead(part, lhs)

    def tail():
        _drain(normalise(NG - 1))
        _drain(combine_w2(0))
        RH = D // 2
        slabs = list(itertools.pairwise([0, 48, 112, 176, RH]))
        b1 = b1_ref[...].astype(F32).reshape(1, F)
        for r0, r1 in slabs:
            lhs = _signed_sums(list(zip(*_OUT)), [hl_s[l * RH + r0:l * RH + r1, j * KB:(j + 1) * KB]
                                                  for j in range(4) for l in range(2)])
            sums = _SignedSums(list(zip(*_LHS)))
            for t in (1, 8, 10, 0, 2, 3, 9, 21, 20, 4, 18, 22, 5, 11, 17, 13, 6, 12, 19, 14, 15, 16, 7):
                sums.feed(t, _dot(lhs[t].astype(BF16), _unpack(wa_s[:, 4 * t * LANE:4 * (t + 1) * LANE])))
            u = sums.result()
            nodes = []
            for l in range(2):
                lo = [u[2 * i + l][:, :FB] for i in range(4)]
                hi = [u[2 * i + l][:, FB:] for i in range(4)]
                h0, h1, h2, h3 = lo[0], hi[1], lo[2], hi[3]
                x = [lo[1], hi[0], lo[3], hi[2], 0.5 * ((h0 + h1) - (h2 + h3)), 0.5 * ((h0 - h1) + (h2 - h3)),
                     0.5 * ((h0 - h1) - (h2 - h3))]
                x = [_gelu(v + b1[:, k * FB:(k + 1) * FB], 1.0 if k < 4 else 0.5) for k, v in enumerate(x)]
                x4, x5, x6 = x[4:]
                nodes.append([jnp.concatenate(pair, axis=1) for pair in (
                    (x4 + x5 + x6, x[1]), (x[0], x4 - x5 - x6), (x5 - x4 - x6, x[3]), (x[2], x6 - x4 - x5))])
            for t, v in enumerate(_signed_sums(_LHS, [nodes[l][i] for i in range(4) for l in range(2)])):
                g_s[r0 // 2:r1 // 2, 4 * t * LANE:4 * (t + 1) * LANE] = _pack(v)
        b2 = b2_ref[...].astype(F32).reshape(1, S)
        copies = []

        def send(rows, cols):
            piece = (pl.ds(rows.start, rows.stop - rows.start), pl.ds(cols.start, cols.stop - cols.start))
            copies.append(pltpu.make_async_copy(out_v.at[piece], out_hbm.at[piece], sems.at[2 * NP + 3]))
            copies[-1].start()

        for q, cuts in ((3, (0, 64, 128, 192, RH)), (2, (0, RH)), (1, (0, RH)), (0, (0, 192, RH))):
            for r0, r1 in itertools.pairwise(cuts):
                sums = _SignedSums(_OUT)
                for t in (1, 0, 8, 9, 2, 3, 10, 22, 4, 20, 17, 18, 21, 5, 11, 12, 6, 16, 7, 19, 13, 14, 15):
                    lhs = _unpack(g_s[r0 // 2:r1 // 2, 4 * t * LANE:4 * (t + 1) * LANE])
                    sums.feed(t, _dot(lhs, weight(wc_s, q, t, FB)))
                    for o, y in sums.finished():
                        rows = slice((o % 2) * RH + r0, (o % 2) * RH + r1)
                        cols = lanes_of(4 * q + o // 2)
                        out_v[rows, cols] = (ht_s[rows, cols] + (y + b2[:, cols])).astype(BF16)
                if q == 0:
                    for l in range(2):
                        send(slice(l * RH + r0, l * RH + r1), slice(0, 4 * LANE))
            if q > 0:
                send(slice(0, D), slice(4 * q * LANE, 4 * (q + 1) * LANE))
        wait_all(copies)

    zero = prologue()
    mem = first_group()
    before_groups(zero)
    lax.fori_loop(1, NG, functools.partial(group, zero), mem)
    tail()


@functools.partial(jax.jit, static_argnames=("A_seg_len",))
def pallas_sequential_preLN__memory_aug_recurrent_mem_tr__mixer_token_mlp__prompt_kernel(
        A_x, A_mem0, A_Wq, A_Wk, A_Wv, A_Wo, A_seg_len, B_x, B_w1, B_b1, B_w2, B_b2):
    del B_x
    _, S, D = A_x.shape
    _, H, E = A_Wq.shape
    M = A_mem0.shape[1]
    F = B_w1.shape[1]
    SEG = int(A_seg_len)
    DP = 512
    NTILE = 56
    hbm = pl.BlockSpec(memory_space=pltpu.HBM)
    vmem = pl.BlockSpec(memory_space=pltpu.VMEM)
    out_t = pl.pallas_call(
        functools.partial(_kernel, S=S, D=D, H=H, E=E, M=M, SEG=SEG, F=F),
        out_shape=jax.ShapeDtypeStruct((D, S), A_x.dtype),
        in_specs=[hbm, vmem, hbm, hbm, hbm, hbm, hbm, vmem, hbm, vmem],
        out_specs=hbm,
        scratch_shapes=[
            pltpu.VMEM((D, S), BF16),
            pltpu.VMEM((H // 2, D, E), U32),
            pltpu.VMEM((H // 2, D, E), U32),
            pltpu.VMEM((H // 2, D, E), U32),
            pltpu.VMEM((H, D, E), BF16),
            pltpu.VMEM((S + 16, F), BF16),
            pltpu.VMEM((F + 16, S), BF16),
            pltpu.VMEM((NTILE * HALF, 7 * LANE), U32),
            pltpu.VMEM((NTILE // 2 * HALF, 23 * LANE), U32),
            pltpu.VMEM((S // 8, 23 * 4 * LANE), U32),
            pltpu.VMEM((S // 512 * F // 7, 23 * LANE), U32),
            pltpu.VMEM((3 * LANE, DP), F32),
            pltpu.VMEM((D, S), F32),
            pltpu.VMEM((D, S), F32),
            pltpu.VMEM((LANE, DP), F32),
            pltpu.VMEM((NTILE // 2 * SEG, len(_AHEAD) * LANE), F32),
            pltpu.VMEM((D, LANE), F32),
            pltpu.VMEM((20 * HALF, DP), U32),
            pltpu.VMEM((20 * HALF, DP), U32),
            pltpu.VMEM((SEG // 2, 23 * LANE), U32),
            pltpu.VMEM((D // 4, 23 * 4 * LANE), U32),
            pltpu.VMEM((D, S), BF16),
            pltpu.SemaphoreType.DMA((H + 4,)),
        ],
        compiler_params=pltpu.CompilerParams(vmem_limit_bytes=120 * 1024 * 1024),
        name="rmt_mixer",
    )(A_x.reshape(S, D).T, A_mem0, A_Wq, A_Wk, A_Wv, A_Wo.transpose(0, 2, 1), B_w1, B_b1, B_w2, B_b2)
    return out_t.T.reshape(1, S, D)
```
